```python
import os as _os
_os.environ.setdefault("JAX_PLATFORMS", "cpu")
import jax
import jax.numpy as jnp

def _softmax(x, axis=-1):
    return jax.nn.softmax(x, axis=axis)
def _gelu(x):
    return jax.nn.gelu(x, approximate=True)
def _silu(x):
    return jax.nn.silu(x)
def _sigmoid(x):
    return jax.nn.sigmoid(x)
def _layernorm(x, axis=-1, eps=1e-5):
    m = jnp.mean(x, axis=axis, keepdims=True)
    v = jnp.var(x, axis=axis, keepdims=True)
    return (x - m) / jnp.sqrt(v + eps)
def _scatter_add(tgt, idx, src, axis=0):
    return tgt.at[idx].add(src)
def _segment_sum(src, seg, n):
    return jax.ops.segment_sum(src, seg, n)
class _Rng:
    def __init__(self, key):
        self._k = key
    def _next(self):
        self._k, sub = jax.random.split(self._k)
        return sub
    def normal(self, shape):
        return jax.random.normal(self._next(), shape, dtype=jnp.bfloat16)
    def randint(self, lo, hi, shape):
        return jax.random.randint(self._next(), shape, lo, hi, dtype=jnp.int32)
    def uniform(self, shape, lo=0.0, hi=1.0):
        return jax.random.uniform(self._next(), shape, jnp.bfloat16, lo, hi)
    def permutation(self, n):
        return jax.random.permutation(self._next(), n)


kernel_name = 'parallel_sum__ssm_conv_h3__dense_activation_silu__prompt'

def setup_inputs():
    _rng = _Rng(jax.random.key(int.from_bytes(__import__("os").urandom(4), "little")))
    _w = (lambda a: (lambda t: t.astype(jnp.bfloat16) if jnp.issubdtype(t.dtype, jnp.floating) else t)(jnp.asarray(a)))
    def _A_setup():
        B, S, D = 1, 2048, 448
        ks = 4
        return {
            "q": _w((lambda *s: _rng.normal(s) * 0.05)(B, S, D)),
            "k": _w((lambda *s: _rng.normal(s) * 0.2)(B, S, D)),
            "v": _w((lambda *s: _rng.normal(s) * 0.2)(B, S, D)),
            "shift_k": _w((lambda *s: _rng.normal(s) * 0.2)(D, ks) * 0.5),
            "ssm_k": _w((lambda *s: _rng.normal(s) * 0.2)(D, S) * (1.0 / S ** 0.5)),
            "ssm_D": _w((lambda *s: _rng.normal(s) * 0.2)(D)),
        }
    _A_in = _A_setup()

    def _B_setup():
        B, S, D, F = 1, 2048, 448, 1792
        return {
            "x": _w((lambda *s: _rng.normal(s) * 0.05)(B, S, D)),
            "w1": _w((lambda *s: _rng.normal(s) * 0.05)(D, F) * (D ** -0.5)),
            "w2": _w((lambda *s: _rng.normal(s) * 0.05)(F, D) * (F ** -0.5)),
        }
    _B_in = _B_setup()

    return {
        "A_q": _A_in["q"],
        "A_k": _A_in["k"],
        "A_v": _A_in["v"],
        "A_shift_k": _A_in["shift_k"],
        "A_ssm_k": _A_in["ssm_k"],
        "A_ssm_D": _A_in["ssm_D"],
        "B_x": _B_in["x"],
        "B_w1": _B_in["w1"],
        "B_w2": _B_in["w2"],
    }

def reference(A_q, A_k, A_v, A_shift_k, A_ssm_k, A_ssm_D, B_x, B_w1, B_w2):
    def _A_ref(q, k, v, shift_k, ssm_k, ssm_D):
        B, S, D = q.shape
        ks = shift_k.shape[-1]
        k_pad = jnp.pad(k, ((0, 0), (ks - 1, 0), (0, 0)))
        k_shift = jnp.zeros_like(k)
        for t in range(ks):
            k_shift = k_shift + k_pad[:, t:t + S, :] * shift_k[:, ks - 1 - t][None, None, :]
        kv = k_shift * v
        L = 2 * S
        kv_pad = jnp.pad(kv, ((0, 0), (0, S), (0, 0)))
        kf_pad = jnp.pad(ssm_k, ((0, 0), (0, S)))
        kv_f = (lambda x, axes=(-2,-1): jnp.fft.rfft2(x.astype(jnp.float32), axes=axes))(kv_pad[:, None, :, :], axes=(1, 2))
        kf_f = (lambda x, axes=(-2,-1): jnp.fft.rfft2(x.astype(jnp.float32), axes=axes))(kf_pad[:, None, :], axes=(1, 2))
        kf_f = (lambda x, *d: x.transpose(*d))(kf_f, 1, 2, 0)
        y_f = kv_f * kf_f[None, :, :, :]
        y = (lambda x, s, axes=(-2,-1): jnp.fft.irfft2(x, s=s, axes=axes).astype(jnp.bfloat16))(y_f, (1, L), axes=(1, 2))[:, 0, :S, :]
        y = y + kv * ssm_D[None, None, :]
        return q * y

    def _B_ref(x, w1, w2):
        h = jnp.einsum("bsd,df->bsf", x, w1)
        h = _silu(h)
        out = jnp.einsum("bsf,fd->bsd", h, w2)
        return out

    x = A_q
    xn = _layernorm(x, axis=-1)
    return x + _A_ref(xn, A_k, A_v, A_shift_k, A_ssm_k, A_ssm_D) + _B_ref(xn, B_w1, B_w2)
```

```python
import numpy as np
import jax
import jax.numpy as jnp
from jax import lax
import jax.experimental.pallas as pl
import jax.experimental.pallas.tpu as pltpu

S, D, FH = 2048, 448, 1792
L = 128
C = S // L
SB = 256
NB = S // SB
G = 64
NG = D // G
FS = 256
NP = FH // FS
EPS = 1e-5
f32, bf16, u32 = jnp.float32, jnp.bfloat16, jnp.uint32
E = lambda k, d: d
REP = int(E("REP", "0"))
NIT = int(E("NIT", str(NB)))
PP = 2
MUL3 = int(E("MUL3", "1"))
FLAGS = None


def _pack_rows(m):
    u = m.astype(bf16).view(np.uint16).astype(np.uint32)
    return (u[1::2] << 16) | u[0::2]


def _consts():
    f = np.arange(L, dtype=np.float64)[:, None]
    b = np.arange(L, dtype=np.float64)[None, :]
    th = np.pi * (2 * f + 1) * b / (2 * L)
    ffwd = np.concatenate([np.cos(th), np.sin(th)], 0)
    ft = ffwd.T
    fi = ffwd * (2.0 / L)
    return _pack_rows(ft.astype(np.float32)), _pack_rows(fi.astype(np.float32))


_FTP, _FIP = _consts()


def kernel(q_hbm, k_hbm, v_hbm, sh_hbm, ssm_hbm, sd_hbm, w1_hbm, w2_hbm, ft_hbm, fi_hbm,
           out_hbm,
           q_v, k_v, v_v, ssm_v, w1_v, w2_v, ft_v, fi_v, sh_v, sd_v,
           xn_s, acc_s, h_s, z_s, kvb_s, xh_s, gh_s, yh_s, o_s, par_s, w1t_s, w2p_s,
           z_smem, sem_q, sem_g, sem_w, sem_out):

    def q_copy(i):
        return pltpu.make_async_copy(q_hbm.at[:, pl.ds(i * SB, SB)], q_v.at[i], sem_q.at[i])

    def g_copies(g):
        r = pl.ds(g * G, G)
        return [
            pltpu.make_async_copy(k_hbm.at[r, :], k_v.at[g], sem_g.at[0, g]),
            pltpu.make_async_copy(v_hbm.at[r, :], v_v.at[g], sem_g.at[1, g]),
            pltpu.make_async_copy(ssm_hbm.at[r, :], ssm_v.at[g], sem_g.at[2, g]),
        ]

    w1_cp = pltpu.make_async_copy(w1_hbm, w1_v, sem_w.at[0])
    w2_cp = pltpu.make_async_copy(w2_hbm, w2_v, sem_w.at[1])
    small = [
        pltpu.make_async_copy(ft_hbm, ft_v, sem_w.at[2]),
        pltpu.make_async_copy(fi_hbm, fi_v, sem_w.at[3]),
        pltpu.make_async_copy(sh_hbm, sh_v, sem_w.at[4]),
        pltpu.make_async_copy(sd_hbm, sd_v, sem_w.at[5]),
    ]

    def out_copy(j):
        return pltpu.make_async_copy(o_s.at[j], out_hbm.at[:, pl.ds(j * SB, SB)], sem_out.at[j])

    for c in small:
        c.start()
    for c in g_copies(0):
        c.start()
    q_copy(0).start()
    w1_cp.start()

    if 0:
        def _zs(j, _):
            z_smem[j] = 0
            return 0
        lax.fori_loop(0, 8, _zs, 0)
    else:
        for i in range(8):
            z_smem[i] = 0

    def opq(base, k, mult=8):
        return pl.multiple_of(base + z_smem[k] * mult, mult)

    for c in small:
        c.wait()
    shf = sh_v[...].astype(f32)
    sdf = 2.0 * sd_v[...].astype(f32)[None, :]
    for j in range(5):
        row = shf[j:j + 1, :] if j < 4 else sdf
        for t in range(4):
            w = min(128, D - t * 128)
            blk = jnp.broadcast_to(row[:, t * 128:t * 128 + w], (128, w))
            if w < 128:
                blk = jnp.concatenate([blk, jnp.zeros((128, 128 - w), f32)], axis=1)
            par_s[j, pl.ds(t * 128, w), :] = blk.T[:w, :]

    st = {}

    def ln1(i, t):
        ls = pl.ds(t * 128, 128)
        tot = None
        for r in range(0, D, 64):
            x = q_v[i, pl.ds(r, 64), ls].astype(f32)
            acc_s[i, pl.ds(r, 64), ls] = x
            tot = x if tot is None else tot + x
        st["m", i, t] = jnp.sum(tot, axis=0, keepdims=True) * (1.0 / D)

    def ln2(i, t):
        ls = pl.ds(t * 128, 128)
        m = st["m", i, t]
        tot = None
        for r in range(0, D, 64):
            xc = acc_s[i, pl.ds(opq(r, 4), 64), ls] - m
            tot = xc * xc if tot is None else tot + xc * xc
        var = jnp.sum(tot, axis=0, keepdims=True) * (1.0 / D)
        st["rs", i, t] = 0.5 * lax.rsqrt(var + EPS)

    def ln3(i, t):
        ls = pl.ds(t * 128, 128)
        m, rs = st["m", i, t], st["rs", i, t]
        for r in range(0, D, 64):
            xn = ((acc_s[i, pl.ds(opq(r, 5), 64), ls] - m) * rs).astype(bf16)
            xn_s[i, pl.ds(r // 2, 32), ls] = pltpu.bitcast(xn, u32)

    def ln_pieces(i):
        out = []
        for fn, cost in ((ln1, 150), (ln2, 180), (ln3, 150)):
            for t in range(2):
                out.append((cost, lambda fn=fn, t=t: fn(i, t)))
        return out

    def mm1(i, p):
        lhs = pltpu.bitcast(w1t_s[pl.ds(p * (FS // 2), FS // 2), :], bf16)
        rhs = pltpu.bitcast(xn_s[i], bf16)
        u = jnp.dot(lhs, rhs, preferred_element_type=f32)
        h = (u + u * jnp.tanh(u)).astype(bf16)
        h_s[pl.ds(p * (FS // 2), FS // 2), :] = pltpu.bitcast(h, u32)

    def mm2(i, p):
        lhs = pltpu.bitcast(w2p_s[:, pl.ds(p * FS, FS)], bf16)
        rhs = pltpu.bitcast(h_s[pl.ds(p * (FS // 2), FS // 2), :], bf16)
        acc_s[i] = acc_s[i] + jnp.dot(lhs, rhs, preferred_element_type=f32)

    lane = lax.broadcasted_iota(jnp.int32, (16, L), 1)
    sgn = jnp.where((lax.broadcasted_iota(jnp.int32, (G, L), 1) & 1) == 0, 1.0, -1.0).astype(f32)

    def prep(g, rb, a0, a1):
        r0 = g * G + rb * 16
        w = [par_s[j, pl.ds(r0, 16), :] for j in range(5)]
        prev = st.get(("rot", g, rb))
        for a in range(a0, a1):
            kc = k_v[g, pl.ds(rb * 16, 16), pl.ds(a * L, L)].astype(f32)
            rot = [pltpu.roll(kc, j, axis=1) for j in range(1, 4)]
            ks = kc * w[0]
            for j in range(1, 4):
                sh = jnp.where(lane >= j, rot[j - 1], 0.0 if prev is None else prev[j - 1])
                ks = ks + sh * w[j]
            prev = rot
            kv = ks * v_v[g, pl.ds(rb * 16, 16), pl.ds(a * L, L)].astype(f32)
            kvb_s[pl.ds(a * (G // 2) + rb * 8, 8), :] = pltpu.bitcast(kv.astype(bf16), u32)
            z_s[pl.ds(r0, 16), pl.ds(a * L, L)] = kv * w[4]
        st["rot", g, rb] = prev

    def dftx(g, qd):
        b = g % 2
        n = C * G // 4
        lhs = pltpu.bitcast(kvb_s[pl.ds(qd * (n // 2), n // 2), :], bf16)
        xh = jnp.dot(lhs, pltpu.bitcast(ft_v[...], bf16), preferred_element_type=f32)
        xh_s[b, pl.ds(qd * n, n), pl.ds(0, 2 * L)] = xh
        if MUL3:
            xh_s[b, pl.ds(qd * n, n), pl.ds(2 * L, L)] = xh[:, :L] + xh[:, L:]

    def dftk(g, qd):
        b = g % 2
        lhs = jnp.concatenate([ssm_v[g, :, pl.ds((4 * qd + c) * L, L)] for c in range(4)], axis=0)
        kh = jnp.dot(lhs, pltpu.bitcast(ft_v[...], bf16), preferred_element_type=f32)
        for c in range(4):
            a = 4 * qd + c
            cur = kh[c * G:(c + 1) * G]
            p = st.get(("kprev", g)) if c == 0 else kh[(c - 1) * G:c * G]
            if p is None:
                gr, gi = cur[:, :L], cur[:, L:]
            else:
                gr = cur[:, :L] + sgn * p[:, L:]
                gi = cur[:, L:] - sgn * p[:, :L]
            gh_s[b, pl.ds(a * G, G), pl.ds(0, L)] = gr
            if MUL3:
                gh_s[b, pl.ds(a * G, G), pl.ds(L, L)] = gi - gr
                gh_s[b, pl.ds(a * G, G), pl.ds(2 * L, L)] = gr + gi
            else:
                gh_s[b, pl.ds(a * G, G), pl.ds(L, L)] = gi
        st["kprev", g] = kh[3 * G:4 * G]

    def mac(g, sg, og):
        b = g % 2
        P = PP
        rr = opq(sg * 8, og % 4)

        def ld(ref, a, part):
            return ref[b, pl.ds(rr + a * G, 8), pl.ds(part * L, L)]

        NM = 3 if MUL3 else 2
        acc = [[None] * NM for _ in range(P)]
        gc = {}
        for ap in range(og * P + P):
            xv = [ld(xh_s, ap, t) for t in range(NM)]
            for o in range(P):
                mm = og * P + o - ap
                if mm < 0:
                    continue
                if mm not in gc:
                    gc[mm] = [ld(gh_s, mm, t) for t in range(NM)]
                gv = gc[mm]
                if MUL3:
                    pr = (gv[0] * xv[2], xv[0] * gv[1], xv[1] * gv[2])
                else:
                    pr = (gv[0] * xv[0] - gv[1] * xv[1], gv[0] * xv[1] + gv[1] * xv[0])
                for t in range(NM):
                    acc[o][t] = pr[t] if acc[o][t] is None else acc[o][t] + pr[t]
        for o in range(P):
            a = og * P + o
            if MUL3:
                re, im = acc[o][0] - acc[o][2], acc[o][0] + acc[o][1]
            else:
                re, im = acc[o]
            yh_s[pl.ds(sg * 8 + a * G, 8), pl.ds(0, L)] = re
            yh_s[pl.ds(sg * 8 + a * G, 8), pl.ds(L, L)] = im

    def inv(g, og):
        n = C * G // 4
        lhs = yh_s[pl.ds(og * n, n), :].astype(bf16)
        y = jnp.dot(lhs, pltpu.bitcast(fi_v[...], bf16), preferred_element_type=f32)
        for c in range(4):
            a = 4 * og + c
            sl = (pl.ds(g * G, G), pl.ds(a * L, L))
            z_s[sl] = z_s[sl] + y[c * G:(c + 1) * G]

    def a_pieces(g):
        out = []
        for half in range(2):
            for rb in range(4):
                out.append((250, lambda rb=rb, half=half: prep(g, rb, half * 8, half * 8 + 8)))
            for qd in (2 * half, 2 * half + 1):
                out.append((60, lambda qd=qd: dftx(g, qd)))
                out.append((220, lambda qd=qd: dftk(g, qd)))
        return out

    def b_pieces(g):
        out = []
        for og in range(C // PP):
            nm = sum(og * PP + o + 1 for o in range(PP))
            for sg in range(G // 8):
                out.append((6 * nm + 2 * PP, lambda sg=sg, og=og: mac(g, sg, og)))
            if ((og + 1) * PP) % 4 == 0:
                out.append((150, lambda og=og: inv(g, ((og + 1) * PP) // 4 - 1)))
        return out

    def comb(j, r):
        o = acc_s[j, pl.ds(r, 64), :] + (
            pltpu.bitcast(xn_s[j, pl.ds(r // 2, 32), :], bf16).astype(f32) * z_s[pl.ds(r, 64), pl.ds(j * SB, SB)])
        o_s[j, pl.ds(r, 64), :] = o.astype(bf16)
        if r + 64 == D:
            out_copy(j).start()

    def comb_pieces(j):
        return [(60, lambda r=r: comb(j, r)) for r in range(0, D, 64)]

    def w1_transpose(p):
        for t in range(FS // 128):
            c0 = p * FS + t * 128
            blk = w1_v[:, pl.ds(c0, 128)]
            w1t_s[pl.ds(c0 // 2, 64), :] = pltpu.bitcast(blk.T, u32)

    def w2_pack(p):
        w2p_s[:, pl.ds(p * FS, FS)] = pltpu.bitcast(w2_v[:, pl.ds(p * FS, FS)], u32)

    def emit(main, sides):
        n = len(main)
        slots = [[] for _ in range(n + 1)]
        for si, (pieces, w0, w1) in enumerate(sides):
            tot = float(sum(c for c, _ in pieces)) or 1.0
            cum = 0.0
            for c, fn in pieces:
                pos = w0 + (cum / tot) * (w1 - w0)
                slots[min(n, int(pos))].append((pos, si, fn))
                cum += c
        for k in range(n + 1):
            for _, _, fn in sorted(slots[k], key=lambda x: (x[0], x[1])):
                fn()
            if k < n:
                main[k]()

    def ffn_main(i):
        order = [("1", 0)]
        for p in range(1, NP):
            order += [("1", p), ("2", p - 1)]
        order.append(("2", NP - 1))
        return [(lambda k=k, p=p: (mm1 if k == "1" else mm2)(i, p)) for k, p in order]

    for c in g_copies(0):
        c.wait()
    w2_cp.start()
    for c in g_copies(1):
        c.start()
    q_copy(1).start()
    for _, fn in a_pieces(0):
        fn()
    q_copy(0).wait()
    for _, fn in ln_pieces(0):
        fn()
    w1_cp.wait()
    for p in range(NP):
        w1_transpose(p)
    w2_cp.wait()
    for p in range(NP):
        w2_pack(p)

    def iteration(i, first_pass=True):
        sides = []
        if first_pass:
            if i + 2 < NG:
                for c in g_copies(i + 2):
                    c.start()
            if i + 2 < NB:
                q_copy(i + 2).start()
            if i + 1 < NG:
                for c in g_copies(i + 1):
                    c.wait()
            if i + 1 < NB:
                q_copy(i + 1).wait()
        if i < NG:
            sides.append((b_pieces(i), 0.0, 14.0))
        if i + 1 < NG:
            sides.append((a_pieces(i + 1), 0.0, 11.0))
        if i + 1 < NB:
            sides.append((ln_pieces(i + 1), 2.0, 8.0))
        if i == NB - 1:
            cp = []
            for j in range(NB - 1):
                cp += comb_pieces(j)
            sides.append((cp, 0.0, 11.0))
        emit(ffn_main(i), sides)

    for i in range(NB):
        iteration(i)
        if REP and i == 3:
            for rep in range(REP):
                iteration(1 + (rep % 2), False)
    for _, fn in comb_pieces(NB - 1):
        fn()
    for j in range(NB):
        out_copy(j).wait()


@jax.jit
def pallas_parallel_sum__ssm_conv_h3__dense_activation_silu__prompt_kernel(
        A_q, A_k, A_v, A_shift_k, A_ssm_k, A_ssm_D, B_x, B_w1, B_w2):
    del B_x
    hbm = pl.BlockSpec(memory_space=pltpu.HBM)
    out = pl.pallas_call(
        kernel,
        out_shape=jax.ShapeDtypeStruct((D, S), bf16),
        in_specs=[hbm] * 10,
        out_specs=hbm,
        scratch_shapes=[
            pltpu.VMEM((NB, D, SB), bf16),
            pltpu.VMEM((NG, G, S), bf16), pltpu.VMEM((NG, G, S), bf16), pltpu.VMEM((NG, G, S), bf16),
            pltpu.VMEM((D, FH), bf16), pltpu.VMEM((D, FH), bf16),
            pltpu.VMEM((L // 2, 2 * L), u32), pltpu.VMEM((L, L), u32),
            pltpu.VMEM((4, D), bf16), pltpu.VMEM((D,), bf16),
            pltpu.VMEM((NB, D // 2, SB), u32),
            pltpu.VMEM((NB, D, SB), f32),
            pltpu.VMEM((FH // 2, SB), u32),
            pltpu.VMEM((D, S), f32),
            pltpu.VMEM((C * G // 2, L), u32),
            pltpu.VMEM((2, C * G, 3 * L), f32),
            pltpu.VMEM((2, C * G, 3 * L), f32),
            pltpu.VMEM((C * G, 2 * L), f32),
            pltpu.VMEM((NB, D, SB), bf16),
            pltpu.VMEM((5, D, L), f32),
            pltpu.VMEM((FH // 2, D), u32),
            pltpu.VMEM((D // 2, FH), u32),
            pltpu.SMEM((8,), jnp.int32),
            pltpu.SemaphoreType.DMA((NB,)),
            pltpu.SemaphoreType.DMA((3, NG)),
            pltpu.SemaphoreType.DMA((6,)),
            pltpu.SemaphoreType.DMA((NB,)),
        ],
        compiler_params=pltpu.CompilerParams(vmem_limit_bytes=64 * 1024 * 1024, flags=FLAGS),
    )(A_q.reshape(S, D).T, A_k.reshape(S, D).T, A_v.reshape(S, D).T, A_shift_k.T, A_ssm_k,
      A_ssm_D, B_w1, B_w2.T, jnp.asarray(_FTP), jnp.asarray(_FIP))
    return out.T.reshape(1, S, D)
```

```python
import numpy as np
import jax
import jax.numpy as jnp
from jax import lax
import jax.experimental.pallas as pl
import jax.experimental.pallas.tpu as pltpu

S, D, FH = 2048, 448, 1792
DP = 512
L = 128
C = S // L
SB = 256
NB = S // SB
G = 64
NG = D // G
FS = 256
NP = FH // FS
EPS = 1e-5
f32, bf16, u32 = jnp.float32, jnp.bfloat16, jnp.uint32
REP = int("0")
PP = int("2")
LOOP = int("3")
FLAGS = None
WB = (0.0, 1.0)
WA = (0.0, 0.75)
WL = "f20 f24".split()
ORD = "abicxd012y3456j"
MG = float("200")
ANCH = int("1")
YP = int("1")
KP = int("0")
M1 = int("896")
SL = int("64")
SK = int("1")
DQ = int("2")
FORD = int("1")
NZ = 512

_off = 0


def _alloc(rows):
    global _off
    b = _off
    _off += rows
    return b


W1_B = _alloc(4 * (FH // 2))
W2_B = _alloc(14 * (D // 2))
YH_B = _alloc(2 * C * G)
KV_B = _alloc(2 * C * G)
POOL_ROWS = _off


def _pack_rows(m):
    u = m.astype(bf16).view(np.uint16).astype(np.uint32)
    return (u[1::2] << 16) | u[0::2]


def _consts():
    f = np.arange(L, dtype=np.float64)[:, None]
    b = np.arange(L, dtype=np.float64)[None, :]
    th = np.pi * (2 * f + 1) * b / (2 * L)
    ffwd = np.concatenate([np.cos(th), np.sin(th)], 0)
    ft = ffwd.T
    fi = ffwd * (2.0 / L)
    return ft.astype(np.float32), fi.astype(np.float32)


_FTP, _FIP = _consts()


def kernel(q_hbm, k_hbm, v_hbm, sh_hbm, ssm_hbm, sd_hbm, w1_hbm, w2_hbm, ft_hbm, fi_hbm,
           out_hbm,
           q_v, k_v, v_v, ssm_v, w1_v, w2_v, ft_v, fi_v, sh_v, sd_v,
           pool, acc_s, h0_s, h1_s, h2_s, h3_s, h4_s, h5_s, h6_s, z_s, xh0_s, gh0_s, xh1_s, gh1_s, yh_s, kv0_s, kv1_s, xn_s, xs_s, o_s, par_s,
           z_smem, sem_q, sem_g, sem_w, sem_out):

    def mo(x, m):
        return x if isinstance(x, int) else pl.multiple_of(x, m)

    def key(x):
        return x if isinstance(x, int) else "dyn"

    def q_copy(i):
        return pltpu.make_async_copy(q_hbm.at[:, pl.ds(mo(i * SB, SB), SB)], q_v.at[i], sem_q.at[i])

    def g_copies(g):
        r = pl.ds(mo(g * G, G), G)
        return [
            pltpu.make_async_copy(k_hbm.at[r, :], k_v.at[g], sem_g.at[0, g]),
            pltpu.make_async_copy(v_hbm.at[r, :], v_v.at[g], sem_g.at[1, g]),
            pltpu.make_async_copy(ssm_hbm.at[r, :], ssm_v.at[g], sem_g.at[2, g]),
        ]

    w1_cp = pltpu.make_async_copy(w1_hbm, w1_v, sem_w.at[0])
    w2_cp = pltpu.make_async_copy(w2_hbm, w2_v, sem_w.at[1])
    small = [
        pltpu.make_async_copy(ft_hbm, ft_v.at[0], sem_w.at[2]),
        pltpu.make_async_copy(fi_hbm, fi_v.at[0], sem_w.at[3]),
        pltpu.make_async_copy(sh_hbm, sh_v, sem_w.at[4]),
        pltpu.make_async_copy(sd_hbm, sd_v, sem_w.at[5]),
    ]

    def out_copy(j):
        return pltpu.make_async_copy(o_s.at[j], out_hbm.at[:, pl.ds(j * SB, SB)], sem_out.at[j])

    for c in small:
        c.start()
    for c in g_copies(0):
        c.start()
    q_copy(0).start()
    w1_cp.start()

    def _zs(j, _):
        z_smem[j] = 0
        return 0
    lax.fori_loop(0, NZ, _zs, 0)

    for i in range(NB):
        for t in range(2):
            xn_s[i, pl.ds(D, DP - D), pl.ds(t * 128, 128)] = jnp.zeros((DP - D, 128), f32)

    for c in small:
        c.wait()
    shf = sh_v[...].astype(f32)
    sdf = 2.0 * sd_v[...].astype(f32)[None, :]
    for j in range(5):
        row = shf[j:j + 1, :] if j < 4 else sdf
        for t in range(4):
            w = min(128, D - t * 128)
            blk = jnp.broadcast_to(row[:, t * 128:t * 128 + w], (128, w))
            if w < 128:
                blk = jnp.concatenate([blk, jnp.zeros((128, 128 - w), f32)], axis=1)
            par_s[j, pl.ds(t * 128, w), :] = blk.T[:w, :]

    st = {"zc": 0}

    def zz():
        st["zc"] = (st["zc"] + 1) % NZ
        return z_smem[st["zc"]]

    def pld(z, row, n):
        return pool[z, pl.ds(row, n), :]

    def as_bf(x):
        return pltpu.bitcast(x, bf16)

    def as_f(x):
        return pltpu.bitcast(x, f32)

    def as_u32(x):
        return pltpu.bitcast(x, u32)

    hs = (h0_s, h1_s, h2_s, h3_s, h4_s, h5_s, h6_s)
    xhs, ghs, kvs = (xh0_s, xh1_s), (gh0_s, gh1_s), (kv0_s, kv1_s)

    def ln1(i, t):
        ls = pl.ds(t * 128, 128)
        tot = None
        for r in range(0, D, 64):
            x = q_v[i, pl.ds(r, 64), ls].astype(f32)
            xs_s[i, pl.ds(r, 64), ls] = x
            tot = x if tot is None else tot + x
        st["m", key(i), t] = jnp.sum(tot, axis=0, keepdims=True) * (1.0 / D)

    def ln2(i, t):
        ls = pl.ds(t * 128, 128)
        m = st["m", key(i), t]
        iz = i + zz()
        tot = None
        for r in range(0, D, 64):
            xc = xs_s[iz, pl.ds(r, 64), ls] - m
            tot = xc * xc if tot is None else tot + xc * xc
        var = jnp.sum(tot, axis=0, keepdims=True) * (1.0 / D)
        st["rs", key(i), t] = 0.5 * lax.rsqrt(var + EPS)

    def ln3(i, t):
        ls = pl.ds(t * 128, 128)
        m, rs = st["m", key(i), t], st["rs", key(i), t]
        iz = i + zz()
        for r in range(0, D, 64):
            xn = (xs_s[iz, pl.ds(r, 64), ls] - m) * rs
            xn_s[i, pl.ds(r, 64), ls] = xn

    def ln_pieces(i):
        out = []
        for fn, cost in ((ln1, 150), (ln2, 180), (ln3, 150)):
            for t in range(2):
                out.append((cost, lambda fn=fn, t=t: fn(i, t)))
        return out

    def m1(i, j, t):
        z0 = zz()
        rhs = xn_s[i + z0, :, pl.ds(t * 128, 128)]
        slabs = []
        for sidx in range(M1 // SL):
            yield
            z = zz()
            slabs.append(jnp.concatenate(
                [pld(z, W1_B + ct * (FH // 2) + j * (M1 // 2) + sidx * (SL // 2), SL // 2) for ct in range(4)], axis=1))
        lhs = as_bf(jnp.concatenate(slabs, axis=0))
        u = jnp.dot(lhs, rhs, preferred_element_type=f32)
        h = u + u * jnp.tanh(u)
        for q_ in range(M1 // 128):
            r = j * M1 + q_ * 128
            p = r // FS
            hs[p][0, pl.ds(r % FS, 128), pl.ds(t * 128, 128)] = h[q_ * 128:(q_ + 1) * 128]

    def m2(i, p):
        z0 = zz()
        rhs = hs[p][z0]
        slabs = []
        for sidx in range(D // SL):
            yield
            z = zz()
            slabs.append(jnp.concatenate(
                [pld(z, W2_B + (2 * p + ct) * (D // 2) + sidx * (SL // 2), SL // 2) for ct in range(2)], axis=1))
        lhs = as_bf(jnp.concatenate(slabs, axis=0))
        acc_s[i] = (xs_s if p == 0 else acc_s)[i + z0] + jnp.dot(lhs, rhs, preferred_element_type=f32)

    lane = lax.broadcasted_iota(jnp.int32, (16, L), 1)
    sgn = jnp.where((lax.broadcasted_iota(jnp.int32, (G, L), 1) & 1) == 0, 1.0, -1.0).astype(f32)


    def prep(g, b, rb, a0, a1):
        r0 = mo(g * G + rb * 16, 16)
        w = [par_s[j, pl.ds(r0, 16), :] for j in range(4)]
        if a0 > 0:
            kp = k_v[g, pl.ds(rb * 16, 16), pl.ds((a0 - 1) * L, L)].astype(f32)
            prev = [pltpu.roll(kp, j, axis=1) for j in range(1, 4)]
        else:
            prev = None
        for a in range(a0, a1):
            kc = k_v[g, pl.ds(rb * 16, 16), pl.ds(a * L, L)].astype(f32)
            rot = [pltpu.roll(kc, j, axis=1) for j in range(1, 4)]
            ks = kc * w[0]
            for j in range(1, 4):
                sh = jnp.where(lane >= j, rot[j - 1], 0.0 if prev is None else prev[j - 1])
                ks = ks + sh * w[j]
            prev = rot
            kv = ks * v_v[g, pl.ds(rb * 16, 16), pl.ds(a * L, L)].astype(f32)
            if KP:
                pool[0, pl.ds(KV_B + b * C * G + a * G + rb * 16, 16), :] = as_u32(kv)
            else:
                kvs[b][0, pl.ds(a * G + rb * 16, 16), :] = kv

    def dftx(g, b, qd):
        xh_s = xhs[b]
        n = C * G // DQ
        zd = zz()
        lhs = as_f(pld(zd, KV_B + b * C * G + qd * n, n)) if KP else kvs[b][zd, pl.ds(qd * n, n), :]
        xh = jnp.dot(lhs, ft_v[zd], preferred_element_type=f32)
        xh_s[0, pl.ds(qd * n, n), pl.ds(0, 2 * L)] = xh
        xh_s[0, pl.ds(qd * n, n), pl.ds(2 * L, L)] = xh[:, :L] + xh[:, L:]

    def dftk(g, b, qd):
        gh_s = ghs[b]
        nc = C // DQ
        lhs = jnp.concatenate([ssm_v[g, :, pl.ds((nc * qd + c) * L, L)] for c in range(nc)], axis=0)
        kh = jnp.dot(lhs, ft_v[zz()], preferred_element_type=f32)
        for c in range(nc):
            a = nc * qd + c
            cur = kh[c * G:(c + 1) * G]
            p = (st.get(("kprev", key(g))) if qd > 0 else None) if c == 0 else kh[(c - 1) * G:c * G]
            if p is None:
                gr, gi = cur[:, :L], cur[:, L:]
            else:
                gr = cur[:, :L] + sgn * p[:, L:]
                gi = cur[:, L:] - sgn * p[:, :L]
            gh_s[0, pl.ds(a * G, G), pl.ds(0, L)] = gr
            gh_s[0, pl.ds(a * G, G), pl.ds(L, L)] = gi - gr
            gh_s[0, pl.ds(a * G, G), pl.ds(2 * L, L)] = gr + gi
        st["kprev", key(g)] = kh[(nc - 1) * G:nc * G]

    def mac(g, b, sg, og):
        P = PP
        bz = zz()
        xh_s, gh_s = xhs[b], ghs[b]

        def ld(ref, a, part):
            return ref[bz, pl.ds(sg * 8 + a * G, 8), pl.ds(part * L, L)]

        acc = [[None] * 3 for _ in range(P)]
        gc = {}
        for ap in range(og * P + P):
            xv = [ld(xh_s, ap, t) for t in range(3)]
            for o in range(P):
                mm = og * P + o - ap
                if mm < 0:
                    continue
                if mm not in gc:
                    gc[mm] = [ld(gh_s, mm, t) for t in range(3)]
                gv = gc[mm]
                pr = (gv[0] * xv[2], xv[0] * gv[1], xv[1] * gv[2])
                for t in range(3):
                    acc[o][t] = pr[t] if acc[o][t] is None else acc[o][t] + pr[t]
        for o in range(P):
            a = og * P + o
            re, im = acc[o][0] - acc[o][2], acc[o][0] + acc[o][1]
            if YP:
                pool[0, pl.ds(YH_B + a * G + sg * 8, 8), :] = pltpu.bitcast(re, u32)
                pool[0, pl.ds(YH_B + C * G + a * G + sg * 8, 8), :] = pltpu.bitcast(im, u32)
            else:
                yh_s[0, pl.ds(a * G + sg * 8, 8), pl.ds(0, L)] = re
                yh_s[0, pl.ds(a * G + sg * 8, 8), pl.ds(L, L)] = im

    def inv(g, b, qd):
        nc = C // DQ // 2
        n = nc * G
        zi = zz()
        fi = fi_v[zi]
        d2 = par_s[4, pl.ds(mo(g * G, G), G), :]
        for hf in range(2):
            r = (2 * qd + hf) * n
            if YP:
                lhs = jnp.concatenate([as_f(pld(zi, YH_B + t * C * G + r, n)) for t in range(2)], axis=1)
            else:
                lhs = yh_s[zi, pl.ds(r, n), :]
            y = jnp.dot(lhs, fi, preferred_element_type=f32)
            for c in range(nc):
                a = nc * (2 * qd + hf) + c
                kv = as_f(pld(zi, KV_B + b * C * G + a * G, G)) if KP else kvs[b][zi, pl.ds(a * G, G), :]
                z_s[pl.ds(mo(g * G, G), G), pl.ds(a * L, L)] = y[c * G:(c + 1) * G] + kv * d2

    def prep_pieces(g, b, hf):
        return [(150, lambda rb=rb, qd=qd: prep(g, b, rb, qd * 4, qd * 4 + 4))
                for qd in (2 * hf, 2 * hf + 1) for rb in range(4)]

    def mac_pieces(g, b, hf):
        out = []
        for og in range(hf * (C // PP // 2), (hf + 1) * (C // PP // 2)):
            nm = sum(og * PP + o + 1 for o in range(PP))
            for sg in range(G // 8):
                out.append((6 * nm + 2 * PP, lambda sg=sg, og=og: mac(g, b, sg, og)))
        return out

    def comb(j, r):
        xn = xn_s[j, pl.ds(r, 64), :]
        o = acc_s[j, pl.ds(r, 64), :] + xn * z_s[pl.ds(r, 64), pl.ds(j * SB, SB)]
        o_s[j, pl.ds(r, 64), :] = o.astype(bf16)
        if r + 64 == D:
            out_copy(j).start()

    def comb_pieces(j):
        return [(60, lambda r=r: comb(j, r)) for r in range(0, D, 64)]

    def w1_transpose(p):
        for t in range(FS // 128):
            c0 = p * FS + t * 128
            blk = w1_v[:, pl.ds(c0, 128)]
            blk = jnp.concatenate([blk, jnp.zeros((DP - D, 128), bf16)], axis=0)
            for ct in range(4):
                pool[0, pl.ds(W1_B + ct * (FH // 2) + c0 // 2, 64), :] = as_u32(blk[ct * 128:(ct + 1) * 128].T)

    def w2_pack(p):
        for ct in range(2):
            c = 2 * p + ct
            pool[0, pl.ds(W2_B + c * (D // 2), D // 2), :] = as_u32(w2_v[:, pl.ds(c * 128, 128)])

    def emit(main, sides):
        t, tstart = 0.0, {}
        for name, _, ns, dt in main:
            tstart[name] = t
            t += ns * dt
        tstart["end"] = t
        items = []
        for pieces, n0, d0, n1, d1 in sides:
            w0, w1 = tstart[n0] + d0, tstart[n1] + d1
            tot = float(sum(c for c, _ in pieces)) or 1.0
            cum = 0.0
            for c, fn in pieces:
                cum += c
                items.append((w0 + (cum / tot) * (w1 - w0), len(items), fn, n1))
        items.sort(key=lambda x: (x[0], x[1]))
        done = set()
        t = 0.0
        for name, gen, ns, dt in main:
            for it_ in items:
                if it_[1] not in done and it_[3] == name:
                    it_[2]()
                    done.add(it_[1])
            if ns == 1 and name[0] == "x":
                gen()
                t += dt
                continue
            it = gen()
            for si in range(ns):
                next(it)
                if si >= SK:
                    for it_ in items:
                        if it_[1] not in done and it_[0] <= t + 1e-6:
                            it_[2]()
                            done.add(it_[1])
                t += dt
            for _ in it:
                pass
        for it_ in items:
            if it_[1] not in done:
                it_[2]()

    for c in g_copies(0):
        c.wait()
    w2_cp.start()
    for c in g_copies(1):
        c.start()
    q_copy(1).start()
    for hf in range(2):
        for _, fn in prep_pieces(0, 0, hf):
            fn()
        dftx(0, 0, hf)
        dftk(0, 0, hf)
    q_copy(0).wait()
    for _, fn in ln_pieces(0):
        fn()
    w1_cp.wait()
    for p in range(NP):
        w1_transpose(p)
    w2_cp.wait()
    for p in range(NP):
        w2_pack(p)

    def iteration(i, first_pass=True, pos=None, par=None):
        par = i % 2 if par is None else par
        pos = i if pos is None else pos
        sides = []
        if first_pass:
            if isinstance(i, int):
                if i + 2 < NG:
                    for c in g_copies(i + 2):
                        c.start()
            else:
                @pl.when(i + 2 < NG)
                def _():
                    for c in g_copies(jnp.minimum(i + 2, NG - 1)):
                        c.start()
            if pos + 2 < NB:
                q_copy(i + 2).start()
            if pos + 1 < NG:
                for c in g_copies(i + 1):
                    c.wait()
            if pos + 1 < NB:
                q_copy(i + 1).wait()
        RS = "bal" if not first_pass else "bal"
        hasb = pos < NG and "b" in RS
        hasa = pos + 1 < NG and "a" in RS
        ga, ba, gb, bb = i + 1, 1 - par, i, par
        F1 = lambda j, t: ("f1%d%d" % (j, t), lambda: m1(i, j, t), M1 // SL, float(SL))
        F2 = lambda p: ("f2%d" % p, lambda: m2(i, p), D // SL, float(SL))
        XI = lambda h: [("xi%d" % h, lambda: inv(gb, bb, h), 1, 256.0)] if hasb else []
        XD = lambda h: [("xd%d" % h, lambda: (dftx(ga, ba, h), dftk(ga, ba, h)), 1, 512.0)] if hasa else []
        tok = dict(a=[F1(0, 0)], b=[F1(0, 1)], c=[F1(1, 0)], d=[F1(1, 1)], i=XI(0), j=XI(1), x=XD(0), y=XD(1))
        for p in range(NP):
            tok[str(p)] = [F2(p)]
        main = sum((tok[ch] for ch in ORD), [])
        if hasb:
            sides.append((mac_pieces(gb, bb, 0), "f100", 0.0, "xi0", -MG))
            sides.append((mac_pieces(gb, bb, 1), "xi0", 0.0, "xi1", -MG))
        if hasa:
            sides.append((prep_pieces(ga, ba, 0), "f100", 0.0, "xd0", -MG))
            sides.append((prep_pieces(ga, ba, 1), "xd0", 256.0, "xd1", -MG))
        if pos + 1 < NB and "l" in RS:
            sides.append((ln_pieces(i + 1), WL[0], 0.0, WL[1], 0.0))
        if pos == NB - 1:
            cp = []
            for j in range(NB - 1):
                cp += comb_pieces(j)
            sides.append((cp, "f100", 0.0, "f25", 0.0))
        emit(main, sides)

    if LOOP:
        def body(j, _):
            iteration(2 * j, True, 0, 0)
            iteration(2 * j + 1, True, 0, 1)
            return 0
        lax.fori_loop(0, LOOP, body, 0)
    for i in range(2 * LOOP, NB):
        iteration(i)
    if REP:
        def body2(i, _):
            iteration(2 * (i % 2), False, 0, 0)
            iteration(2 * (i % 2) + 1, False, 0, 1)
            return 0
        lax.fori_loop(0, REP, body2, 0)
    for _, fn in comb_pieces(NB - 1):
        fn()
    for j in range(NB):
        out_copy(j).wait()


@jax.jit
def pallas_parallel_sum__ssm_conv_h3__dense_activation_silu__prompt_kernel(
        A_q, A_k, A_v, A_shift_k, A_ssm_k, A_ssm_D, B_x, B_w1, B_w2):
    del B_x
    hbm = pl.BlockSpec(memory_space=pltpu.HBM)
    out = pl.pallas_call(
        kernel,
        out_shape=jax.ShapeDtypeStruct((D, S), bf16),
        in_specs=[hbm] * 10,
        out_specs=hbm,
        scratch_shapes=[
            pltpu.VMEM((NB, D, SB), bf16),
            pltpu.VMEM((NG, G, S), bf16), pltpu.VMEM((NG, G, S), bf16), pltpu.VMEM((NG, G, S), bf16),
            pltpu.VMEM((D, FH), bf16), pltpu.VMEM((D, FH), bf16),
            pltpu.VMEM((1, L, 2 * L), f32), pltpu.VMEM((1, 2 * L, L), f32),
            pltpu.VMEM((4, D), bf16), pltpu.VMEM((D,), bf16),
            pltpu.VMEM((1, POOL_ROWS, 128), u32),
            pltpu.VMEM((NB, D, SB), f32),
            *[pltpu.VMEM((1, FS, SB), f32)] * NP,
            pltpu.VMEM((D, S), f32),
            pltpu.VMEM((1, C * G, 3 * L), f32), pltpu.VMEM((1, C * G, 3 * L), f32),
            pltpu.VMEM((1, C * G, 3 * L), f32), pltpu.VMEM((1, C * G, 3 * L), f32),
            pltpu.VMEM((1, C * G, 2 * L), f32),
            pltpu.VMEM((1, C * G, L), f32), pltpu.VMEM((1, C * G, L), f32),
            pltpu.VMEM((NB, DP, SB), f32),
            pltpu.VMEM((NB, D, SB), f32),
            pltpu.VMEM((NB, D, SB), bf16),
            pltpu.VMEM((5, D, L), f32),
            pltpu.SMEM((NZ,), jnp.int32),
            pltpu.SemaphoreType.DMA((NB,)),
            pltpu.SemaphoreType.DMA((3, NG)),
            pltpu.SemaphoreType.DMA((6,)),
            pltpu.SemaphoreType.DMA((NB,)),
        ],
        compiler_params=pltpu.CompilerParams(vmem_limit_bytes=64 * 1024 * 1024, flags=FLAGS),
    )(A_q.reshape(S, D).T, A_k.reshape(S, D).T, A_v.reshape(S, D).T, A_shift_k.T, A_ssm_k,
      A_ssm_D, B_w1, B_w2.T, jnp.asarray(_FTP), jnp.asarray(_FIP))
    return out.T.reshape(1, S, D)
```
